```python
import jax
import jax.numpy as jnp

def _softmax(x, axis=-1):
    return jax.nn.softmax(x, axis=axis)
def _gelu(x):
    return jax.nn.gelu(x, approximate=True)
def _silu(x):
    return jax.nn.silu(x)
def _sigmoid(x):
    return jax.nn.sigmoid(x)
def _layernorm(x, axis=-1, eps=1e-5):
    m = jnp.mean(x, axis=axis, keepdims=True)
    v = jnp.var(x, axis=axis, keepdims=True)
    return (x - m) / jnp.sqrt(v + eps)
def _scatter_add(tgt, idx, src, axis=0):
    return tgt.at[idx].add(src)
def _segment_sum(src, seg, n):
    return jax.ops.segment_sum(src, seg, n)
class _Rng:
    def __init__(self, key):
        self._k = key
    def _next(self):
        self._k, sub = jax.random.split(self._k)
        return sub
    def normal(self, shape):
        return jax.random.normal(self._next(), shape, dtype=jnp.bfloat16)
    def randint(self, lo, hi, shape):
        return jax.random.randint(self._next(), shape, lo, hi, dtype=jnp.int32)
    def uniform(self, shape, lo=0.0, hi=1.0):
        return jax.random.uniform(self._next(), shape, jnp.bfloat16, lo, hi)
    def permutation(self, n):
        return jax.random.permutation(self._next(), n)


kernel_name = 'concat_heads__sliding_block_cached__compressed_kv_cla__decode'

def _fwd_setup_inputs():
    _rng = _Rng(jax.random.key(int.from_bytes(__import__("os").urandom(4), "little")))
    _w = (lambda a: (lambda t: t.astype(jnp.bfloat16) if jnp.issubdtype(t.dtype, jnp.floating) else t)(jnp.asarray(a)))
    def _A_setup():
        B, Sq, D = 1, 1, 640
        Hq, Hkv, Sk, Dh = 32, 32, 4096, 128
        assert Hq % Hkv == 0, (Hq, Hkv)
        return {
            "x": _w((lambda *s: _rng.normal(s) * 0.05)(B, Sq, D)),
            "k_cache": _w((lambda *s: _rng.normal(s) * 0.05)(B, Hkv, Sk, Dh)),
            "v_cache": _w((lambda *s: _rng.normal(s) * 0.05)(B, Hkv, Sk, Dh)),
            "wq": _w((lambda *s: _rng.normal(s) * 0.05)(D, Hq * Dh) * (D ** -0.5)),
            "wo": _w((lambda *s: _rng.normal(s) * 0.05)(Hq * Dh, D) * ((Hq * Dh) ** -0.5)),
        }
    _A_in = _A_setup()

    def _B_setup():
        B, H, Sq, Sk, D, M = 1, 32, 1, 4096, 128, 640
        Dc = 4 * D
        return {
            "x": _w((lambda *s: _rng.normal(s) * 0.05)(B, Sq, M)),
            "c_kv": _w((lambda *s: _rng.normal(s) * 0.05)(B, Sk, Dc)),
            "w_q": _w((lambda *s: _rng.normal(s) * 0.05)(M, H, D) * (M ** -0.5)),
            "w_uk": _w((lambda *s: _rng.normal(s) * 0.05)(Dc, H, D) * (Dc ** -0.5)),
            "w_uv": _w((lambda *s: _rng.normal(s) * 0.05)(Dc, H, D) * (Dc ** -0.5)),
            "w_o": _w((lambda *s: _rng.normal(s) * 0.05)(H, D, M) * ((H * D) ** -0.5)),
        }
    _B_in = _B_setup()

    return {
        "A_x": _A_in["x"],
        "A_k_cache": _A_in["k_cache"],
        "A_v_cache": _A_in["v_cache"],
        "A_wq": _A_in["wq"],
        "A_wo": _A_in["wo"],
        "B_x": _B_in["x"],
        "B_c_kv": _B_in["c_kv"],
        "B_w_q": _B_in["w_q"],
        "B_w_uk": _B_in["w_uk"],
        "B_w_uv": _B_in["w_uv"],
        "B_w_o": _B_in["w_o"],
    }

def _fwd_reference(A_x, A_k_cache, A_v_cache, A_wq, A_wo, B_x, B_c_kv, B_w_q, B_w_uk, B_w_uv, B_w_o):
    def _A_ref(x, k_cache, v_cache, wq, wo):
        B, Sq, D = x.shape
        Hq, Dh = 32, 128
        Hkv, Sk = k_cache.shape[1], k_cache.shape[2]
        W = min(4096, max(256, Sk // 4))
        rep = Hq // Hkv
        q = (lambda x, *d: x.transpose(*d))((x @ wq).reshape(B, Sq, Hq, Dh), 0, 2, 1, 3)
        k = jnp.repeat(k_cache[:, :, Sk - W:, :], rep, axis=1)
        v = jnp.repeat(v_cache[:, :, Sk - W:, :], rep, axis=1)
        scores = jnp.einsum("bhqd,bhkd->bhqk", q, k) * (Dh ** -0.5)
        p = _softmax(scores, axis=-1)
        o = jnp.einsum("bhqk,bhkd->bhqd", p, v)
        return (lambda x, *d: x.transpose(*d))(o, 0, 2, 1, 3).reshape(B, Sq, Hq * Dh) @ wo

    def _B_ref(x, c_kv, w_q, w_uk, w_uv, w_o):
        B, Sq, M = x.shape[0], x.shape[1], x.shape[2]
        Sk = c_kv.shape[1]
        H, D = w_q.shape[1], w_q.shape[2]
        q = jnp.einsum("bqm,mhd->bhqd", x, w_q)
        k = jnp.einsum("bkc,chd->bhkd", c_kv, w_uk)
        v = jnp.einsum("bkc,chd->bhkd", c_kv, w_uv)
        scores = jnp.einsum("bhqd,bhkd->bhqk", q, k) * (D ** -0.5)
        off = Sk - Sq
        qi = jnp.arange(Sq)[:, None]
        kj = jnp.arange(Sk)[None, :]
        cmask = kj <= (qi + off)
        scores = jnp.where(cmask[None, None], scores, -1e9)
        p = _softmax(scores, axis=-1)
        ctx = jnp.einsum("bhqk,bhkd->bhqd", p, v)
        return jnp.einsum("bhqd,hdm->bqm", ctx, w_o)

    a = _A_ref(A_x, A_k_cache, A_v_cache, A_wq, A_wo)
    b = _B_ref(B_x, B_c_kv, B_w_q, B_w_uk, B_w_uv, B_w_o)
    return jnp.concatenate([a, b], axis=-1)


def setup_inputs():
    _inp = _fwd_setup_inputs()
    _gk = jax.random.fold_in(jax.random.key(int.from_bytes(__import__("os").urandom(4), "little")), 2**31 - 1)
    _shapes = [[1, 1, 1280]]
    _dtypes = ['bfloat16']
    _gks = jax.random.split(_gk, len(_shapes))
    _gs = [jax.random.normal(k, s, dtype=jnp.dtype(d)) * 0.05 for k, s, d in zip(_gks, _shapes, _dtypes)]
    _inp["grad_out"] = _gs[0]
    return _inp

def reference(A_x, A_k_cache, A_v_cache, A_wq, A_wo, B_x, B_c_kv, B_w_q, B_w_uk, B_w_uv, B_w_o, grad_out):
    _const = dict()
    def _f(*_d):
        return _fwd_reference(**{'A_x': _d[0], 'A_k_cache': _d[1], 'A_v_cache': _d[2], 'A_wq': _d[3], 'A_wo': _d[4], 'B_x': _d[5], 'B_c_kv': _d[6], 'B_w_q': _d[7], 'B_w_uk': _d[8], 'B_w_uv': _d[9], 'B_w_o': _d[10], **_const})
    _out, _vjp = jax.vjp(_f, A_x, A_k_cache, A_v_cache, A_wq, A_wo, B_x, B_c_kv, B_w_q, B_w_uk, B_w_uv, B_w_o)
    _grads = _vjp(grad_out)
    _out0 = jnp.asarray(_out)
    return (_out0, *[jnp.asarray(_g) for _g in _grads])
```

```python
import jax
import jax.numpy as jnp
from jax import lax
import jax.experimental.pallas as pl
import jax.experimental.pallas.tpu as pltpu

F32 = jnp.float32
BF16 = jnp.bfloat16

H = 32
D = 128
SK = 4096
WIN = 1024
M = 640
C = 512
HD = H * D
SCALE = float(D) ** -0.5

KV_GROUPS = 8
HPG = H // KV_GROUPS

CFG = dict(
    ckv_split=3072,
    wq=(10, 8, 2048),
    wo=(8, 32),
    ckv=(8, 32),
    bwq=(10, 128),
    bwu=(8, 128),
    order=("gv", "gckv", "gbwuk", "gbwuv", "gbwo", "gbwq", "gawo", "gawq"),
)

ZR = 128
ZJ = 8
NZB = (SK - WIN) // ZR
NDB = WIN // ZR
NHG = H // ZJ

NT = (((1,), (1,)), ((), ()))


def _dot(a, b):
    return jnp.dot(a, b, preferred_element_type=F32)


def _dot_nt(a, b):
    return lax.dot_general(a, b, NT, preferred_element_type=F32)


def _iota(shape, dim):
    return lax.broadcasted_iota(jnp.int32, shape, dim)


def _colrep(row):
    eye = _iota((128, 128), 0) == _iota((128, 128), 1)
    lhs = jnp.where(eye, jnp.broadcast_to(row, (128, 128)), 0.0).astype(BF16)
    return _dot(lhs, jnp.ones((128, 128), BF16))


def _kernel(
    ax_h, ak_h, av_h, awq_h, awo_h, bx_h, ckv_h, bwq_h, bwuk_h, bwuv_h, bwo_h, g_h,
    out_h, gax_h, gak_h, gav_h, gawq_h, gawo_h, gbx_h, gckv_h, gbwq_h, gbwuk_h, gbwuv_h, gbwo_h,
    ax_v, bx_v, g_v, k_v, v_v, awq_v, awo_v, ckv_v, bwq_v, bwuk_v, bwuv_v, bwo_v,
    out_s, gax_s, gbx_s, z_s, gk_s, gv_s, gawq_s, gawo_s, gckv_s, gbwq_s, gbwuk_s, gbwuv_s, gbwo_s,
    qa_s, doa_s, oa_s, dqa_s, qb_s, dctx_s, ctx_s, dqb_s, row_s, xrep_s, t3_s, qd_s, ps_s, latt_s,
    rsem, wsem,
):
    CKV_SPLIT = CFG["ckv_split"]
    reads = {}

    def add_read(name, src, dst):
        reads[name] = pltpu.make_async_copy(src, dst, rsem.at[len(reads)])

    add_read("awq", awq_h, awq_v)
    add_read("ax", ax_h, ax_v)
    add_read("bx", bx_h, bx_v)
    add_read("g", g_h, g_v)
    add_read("awo", awo_h, awo_v)
    for gi in range(KV_GROUPS):
        hs = pl.ds(gi * HPG, HPG)
        add_read(("k", gi), ak_h.at[hs, pl.ds(SK - WIN, WIN), :], k_v.at[hs])
        add_read(("v", gi), av_h.at[hs, pl.ds(SK - WIN, WIN), :], v_v.at[hs])
    add_read("bwq", bwq_h, bwq_v)
    add_read("bwo", bwo_h, bwo_v)
    add_read("bwuk", bwuk_h, bwuk_v)
    add_read("bwuv", bwuv_h, bwuv_v)
    add_read("ckv0", ckv_h.at[pl.ds(0, CKV_SPLIT)], ckv_v.at[pl.ds(0, CKV_SPLIT)])
    add_read("ckv1", ckv_h.at[pl.ds(CKV_SPLIT, SK - CKV_SPLIT)], ckv_v.at[pl.ds(CKV_SPLIT, SK - CKV_SPLIT)])

    def zero_copy(dst_h, i):
        hg = i // NZB
        rb = i % NZB
        return pltpu.make_async_copy(
            z_s, dst_h.at[pl.ds(hg * ZJ, ZJ), pl.ds(pl.multiple_of(rb * ZR, ZR), ZR), :], wsem.at[0])

    def cache_copy(src, dst_h, i):
        hg = i // NDB
        r0 = pl.multiple_of((i % NDB) * ZR, ZR)
        return pltpu.make_async_copy(
            src.at[pl.ds(hg * ZJ, ZJ), pl.ds(r0, ZR), :],
            dst_h.at[pl.ds(hg * ZJ, ZJ), pl.ds(pl.multiple_of(SK - WIN + r0, ZR), ZR), :], wsem.at[1])

    def rows_copy(src, dst_h, rows, sem_i):
        def mk(i):
            r0 = pl.multiple_of(i * rows, rows)
            return pltpu.make_async_copy(src.at[:, pl.ds(r0, rows), :], dst_h.at[:, pl.ds(r0, rows), :],
                                         wsem.at[sem_i])
        return mk, src.shape[1] // rows

    _, wq_r, wq_c = CFG["wq"]
    wq_nc = HD // wq_c

    def wq_copy(i):
        r0 = pl.multiple_of((i // wq_nc) * wq_r, wq_r)
        c0 = pl.multiple_of((i % wq_nc) * wq_c, wq_c)
        return pltpu.make_async_copy(gawq_s.at[:, pl.ds(r0, wq_r), pl.ds(c0, wq_c)],
                                     gawq_h.at[:, pl.ds(r0, wq_r), pl.ds(c0, wq_c)], wsem.at[2])

    writes = {
        "z": (lambda i: zero_copy(gak_h, i), NHG * NZB),
        "zv": (lambda i: zero_copy(gav_h, i), NHG * NZB),
        "gk": (lambda i: cache_copy(gk_s, gak_h, i), NHG * NDB),
        "gv": (lambda i: cache_copy(gv_s, gav_h, i), NHG * NDB),
        "gawq": (wq_copy, (gawq_s.shape[1] // wq_r) * wq_nc),
        "gawo": rows_copy(gawo_s, gawo_h, CFG["wo"][1], 3),
        "gckv": rows_copy(gckv_s, gckv_h, CFG["ckv"][1], 4),
        "gbwq": rows_copy(gbwq_s, gbwq_h, CFG["bwq"][1], 5),
        "gbwuk": rows_copy(gbwuk_s, gbwuk_h, CFG["bwu"][1], 6),
        "gbwuv": rows_copy(gbwuv_s, gbwuv_h, CFG["bwu"][1], 6),
        "gbwo": rows_copy(gbwo_s, gbwo_h, CFG["wo"][1], 3),
    }
    issued = {name: 0 for name in writes}

    def issue(name, count=None):
        mk, n = writes[name]
        lo = issued[name]
        hi = n if count is None else lo + count
        assert hi <= n
        issued[name] = hi

        def body(i, carry):
            mk(i).start()
            return carry
        lax.fori_loop(lo, hi, body, 0)

    def wait_writes(name):
        mk, n = writes[name]
        assert issued[name] == n

        def body(i, carry):
            mk(i).wait()
            return carry
        lax.fori_loop(0, n, body, 0)

    small_writes = [
        pltpu.make_async_copy(out_s, out_h, wsem.at[7]),
        pltpu.make_async_copy(gax_s, gax_h, wsem.at[8]),
        pltpu.make_async_copy(gbx_s, gbx_h, wsem.at[9]),
    ]

    def xa():
        return ax_v[0].astype(F32)

    def xb():
        return bx_v[0].astype(F32)

    def ga():
        return g_v[0][:, :M].astype(F32)

    def gb():
        return g_v[0][:, M:].astype(F32)

    def put_rows(dst, r, n, val, cols=None):
        rps = dst.shape[1]
        seg = r // rps
        r0 = r % rps
        if not isinstance(r0, int):
            r0 = pl.multiple_of(r0, n)
        if cols is None:
            dst[seg, pl.ds(r0, n), :] = val
        else:
            dst[seg, pl.ds(r0, n), cols] = val

    def rows16(row):
        return jnp.broadcast_to(row, (16, row.shape[1])).astype(BF16)

    def row_to_heads(row, dst):
        for h in range(H):
            dst[h:h + 1, :] = row[0:1, h * D:(h + 1) * D]

    def heads_to_row(src):
        for h in range(H):
            row_s[:, h * D:(h + 1) * D] = jnp.broadcast_to(src[h:h + 1, :], (16, D)).astype(BF16)
        return row_s[...]

    def fill_xrep(x):
        for t in range(M // 128):
            xrep_s[t * 128:(t + 1) * 128, :] = _colrep(x[:, t * 128:(t + 1) * 128])

    def outer_wo(src, grow, dst):
        def body(h, carry):
            col = _colrep(src[pl.ds(h, 1), :])
            for t in range(M // 128):
                put_rows(dst, h * D, D, (col * grow[:, t * 128:(t + 1) * 128]).astype(BF16),
                         slice(t * 128, (t + 1) * 128))
            return carry
        lax.fori_loop(0, H, body, 0)

    def a_q():
        row_to_heads(_dot(rows16(xa()), awq_v[...]), qa_s)

    def a_do():
        row_to_heads(_dot_nt(rows16(ga()), awo_v[...]), doa_s)

    def a_head(h, carry):
        kk = k_v[h]
        vv = v_v[h]
        q = qa_s[pl.ds(h, 1), :]
        do = doa_s[pl.ds(h, 1), :]
        s = _dot_nt(kk, jnp.broadcast_to(q, (D, D)).astype(BF16)) * SCALE
        dp = _dot_nt(vv, jnp.broadcast_to(do, (D, D)).astype(BF16))
        mx = jnp.max(s, axis=0, keepdims=True)
        e = jnp.exp(s - mx)
        inv = 1.0 / jnp.sum(e, axis=0, keepdims=True)
        cc = jnp.sum(e * dp, axis=0, keepdims=True) * inv
        u = e * (dp - cc)
        f = inv * SCALE
        gk_s[h] = (u * (q * f)).astype(BF16)
        gv_s[h] = (e * (do * inv)).astype(BF16)
        oa_s[pl.ds(h, 1), :] = jnp.sum(e * vv.astype(F32), axis=0, keepdims=True) * inv
        dqa_s[pl.ds(h, 1), :] = jnp.sum(u * kk.astype(F32), axis=0, keepdims=True) * f
        return carry

    def a_out():
        out_s[0, :, 0:M] = _dot(heads_to_row(oa_s), awo_v[...])[0:1].astype(BF16)

    def a_dwo():
        outer_wo(oa_s, ga(), gawo_s)

    def a_dx():
        gax_s[0] = _dot_nt(heads_to_row(dqa_s), awq_v[...])[0:1].astype(BF16)

    def a_dwq():
        fill_xrep(xa())
        for h in range(H):
            blk = (xrep_s[...] * dqa_s[h:h + 1, :]).astype(BF16)
            gawq_s[:, :, h * D:(h + 1) * D] = blk.reshape(gawq_s.shape[0], gawq_s.shape[1], D)

    def b_q():
        fill_xrep(xb())

        def body(i, acc):
            for j in range(8):
                m = i * 8 + j
                w = bwq_v[pl.ds(pl.multiple_of(m * H, H), H), :].astype(F32)
                acc = acc + w * xrep_s[pl.ds(m, 1), :]
            return acc
        qb_s[...] = lax.fori_loop(0, M // 8, body, jnp.zeros((H, D), F32))

    def b_dctx():
        row_to_heads(_dot_nt(rows16(gb()), bwo_v[...]), dctx_s)

    def b_absorb(w_v, vec_s, first):
        cb = 16
        diag = (_iota((cb * H, D), 0) % H) == (_iota((cb * H, D), 1) % H)
        zpad = jnp.zeros((H, D), F32)
        parts = [vec_s[...], zpad, zpad, zpad] if first else [zpad, vec_s[...], zpad, zpad]
        rhs = jnp.concatenate(parts, axis=0).astype(BF16)

        def body(i, carry):
            r0 = pl.multiple_of(i * cb * H, cb * H)
            r = _dot_nt(w_v[pl.ds(r0, cb * H), :], rhs)
            r = jnp.where(diag, r, 0.0).reshape(cb, 4, 8, D)
            r = (r[:, 0] + r[:, 1]) + (r[:, 2] + r[:, 3])
            r = r.reshape(cb * 8, D)
            t0 = pl.multiple_of(i * cb * 8, cb * 8)
            if first:
                t3_s[pl.ds(t0, cb * 8), :] = r
            else:
                t3_s[pl.ds(t0, cb * 8), :] = t3_s[pl.ds(t0, cb * 8), :] + r
            return carry
        lax.fori_loop(0, C // cb, body, 0)

    def b_qd():
        qdt = t3_s[pl.ds(0, C, stride=8), :]
        for i in range(1, 8):
            qdt = qdt + t3_s[pl.ds(i, C, stride=8), :]
        qd_s[...] = qdt.T.astype(BF16)

    def b_attn():
        sd = _dot_nt(qd_s[0:64, :], ckv_v[...])
        s = sd[0:H] * SCALE
        dp = sd[H:2 * H]
        e = jnp.exp(s - jnp.max(s, axis=1, keepdims=True))
        p = e * (1.0 / jnp.sum(e, axis=1, keepdims=True))
        ds = p * (dp - jnp.sum(p * dp, axis=1, keepdims=True)) * SCALE
        ps_s[0:H, :] = ds
        ps_s[H:2 * H, :] = p
        ps_s[2 * H:4 * H, :] = jnp.zeros((2 * H, SK), F32)
        lat = _dot(ps_s[...].astype(BF16), ckv_v[...])
        latt_s[...] = lat.T

    def b_dckv():
        def body(j, carry):
            k0 = pl.multiple_of(j * 512, 512)
            pst = ps_s[:, pl.ds(k0, 512)].T.astype(BF16)
            put_rows(gckv_s, j * 512, 512, _dot(pst, qd_s[...]).astype(BF16))
            return carry
        lax.fori_loop(0, SK // 512, body, 0)

    def b_lat():
        cc = 8
        sel = (_iota((cc * H, D), 0) % H) == (_iota((cc * H, D), 1) % H)
        jj = _iota((D, 2 * D), 0)
        nn = _iota((D, 2 * D), 1)
        expand = jnp.where(((jj < H) & (nn < D)) | ((jj >= H) & (jj < 2 * H) & (nn >= D)), 1.0, 0.0).astype(BF16)
        qb_t = jnp.concatenate([qb_s[...]] * cc, axis=0)
        dctx_t = jnp.concatenate([dctx_s[...]] * cc, axis=0)

        def body(i, carry):
            dq_acc, ctx_acc = carry
            c0 = i * cc
            lhs = jnp.concatenate(
                [jnp.broadcast_to(latt_s[pl.ds(c0 + j, 1), :], (H, D)) for j in range(cc)], axis=0)
            rep = _dot(jnp.where(sel, lhs, 0.0).astype(BF16), expand)
            rep_ds = rep[:, 0:D]
            rep_p = rep[:, D:2 * D]
            r0 = pl.multiple_of(c0 * H, cc * H)
            put_rows(gbwuk_s, c0 * H, cc * H, (rep_ds * qb_t).astype(BF16))
            put_rows(gbwuv_s, c0 * H, cc * H, (rep_p * dctx_t).astype(BF16))
            wk = bwuk_v[pl.ds(r0, cc * H), :].astype(F32)
            wv = bwuv_v[pl.ds(r0, cc * H), :].astype(F32)
            dq_acc = dq_acc + jnp.sum((rep_ds * wk).reshape(cc, H, D), axis=0)
            ctx_acc = ctx_acc + jnp.sum((rep_p * wv).reshape(cc, H, D), axis=0)
            return dq_acc, ctx_acc

        dqb, ctx = lax.fori_loop(0, C // cc, body, (jnp.zeros((H, D), F32), jnp.zeros((H, D), F32)))
        ctx_s[...] = ctx
        dqb_s[...] = dqb

    def b_out():
        out_s[0, :, M:2 * M] = _dot(heads_to_row(ctx_s), bwo_v[...])[0:1].astype(BF16)

    def b_dwo():
        outer_wo(ctx_s, gb(), gbwo_s)

    def b_dwq():
        def body(i, carry):
            dq = dqb_s[...]
            for j in range(8):
                m = i * 8 + j
                w = bwq_v[pl.ds(pl.multiple_of(m * H, H), H), :].astype(F32) * dq
                t3_s[pl.ds(pl.multiple_of(m * 8, 8), 8), :] = (w[0:8] + w[8:16]) + (w[16:24] + w[24:32])
                put_rows(gbwq_s, m * H, H, (xrep_s[pl.ds(m, 1), :] * dq).astype(BF16))
            return carry
        lax.fori_loop(0, M // 8, body, 0)
        tt = t3_s[pl.ds(0, M, stride=8), :]
        for i in range(1, 8):
            tt = tt + t3_s[pl.ds(i, M, stride=8), :]
        gbx_s[0] = jnp.sum(tt.T, axis=0, keepdims=True).astype(BF16)

    for cp in reads.values():
        cp.start()
    z_s[...] = jnp.zeros(z_s.shape, BF16)

    reads["ax"].wait()
    reads["bx"].wait()
    reads["g"].wait()
    reads["awq"].wait()
    a_q()
    reads["awo"].wait()
    a_do()
    for gi in range(KV_GROUPS):
        reads[("k", gi)].wait()
        reads[("v", gi)].wait()
        lax.fori_loop(gi * HPG, (gi + 1) * HPG, a_head, 0)
    reads["bwq"].wait()
    b_q()
    reads["bwo"].wait()
    b_dctx()
    reads["bwuk"].wait()
    b_absorb(bwuk_v, qb_s, True)
    reads["bwuv"].wait()
    reads["ckv0"].wait()
    issue("z", 72)
    b_absorb(bwuv_v, dctx_s, False)
    b_qd()
    reads["ckv1"].wait()
    b_attn()
    issue("z")
    issue("zv", 16)
    b_dckv()
    issue("zv", 16)
    b_lat()
    issue("zv", 40)
    b_out()
    b_dwo()
    issue("zv")
    b_dwq()
    issue("gk", 16)
    a_out()
    a_dwo()
    issue("gk")
    a_dx()
    a_dwq()
    for cp in small_writes:
        cp.start()
    for name in CFG["order"]:
        issue(name)

    for name in ("z", "zv", "gk"):
        wait_writes(name)
    for cp in small_writes:
        cp.wait()
    for name in CFG["order"]:
        wait_writes(name)


@jax.jit
def pallas_concat_heads__sliding_block_cached__compressed_kv_cla__decode_kernel(
    A_x: jax.Array,
    A_k_cache: jax.Array,
    A_v_cache: jax.Array,
    A_wq: jax.Array,
    A_wo: jax.Array,
    B_x: jax.Array,
    B_c_kv: jax.Array,
    B_w_q: jax.Array,
    B_w_uk: jax.Array,
    B_w_uv: jax.Array,
    B_w_o: jax.Array,
    grad_out: jax.Array,
):
    sds = jax.ShapeDtypeStruct
    jq, jo, jc, jbq, jbu = (CFG[k][0] for k in ("wq", "wo", "ckv", "bwq", "bwu"))
    s_wq = (jq, M // jq, HD)
    s_wo = (jo, HD // jo, M)
    s_ckv = (jc, SK // jc, C)
    s_bwq = (jbq, M * H // jbq, D)
    s_bwu = (jbu, C * H // jbu, D)
    out_shape = (
        sds((1, 1, 2 * M), BF16),
        sds((1, 1, M), BF16),
        sds((H, SK, D), BF16),
        sds((H, SK, D), BF16),
        sds(s_wq, BF16),
        sds(s_wo, BF16),
        sds((1, 1, M), BF16),
        sds(s_ckv, BF16),
        sds(s_bwq, BF16),
        sds(s_bwu, BF16),
        sds(s_bwu, BF16),
        sds(s_wo, BF16),
    )
    vm = pltpu.VMEM
    scratch = [
        vm((1, 1, M), BF16), vm((1, 1, M), BF16), vm((1, 1, 2 * M), BF16),
        vm((H, WIN, D), BF16), vm((H, WIN, D), BF16),
        vm((M, HD), BF16), vm((HD, M), BF16),
        vm((SK, C), BF16),
        vm((M * H, D), BF16), vm((C * H, D), BF16), vm((C * H, D), BF16), vm((HD, M), BF16),
        vm((1, 1, 2 * M), BF16), vm((1, 1, M), BF16), vm((1, 1, M), BF16),
        vm((ZJ, ZR, D), BF16),
        vm((H, WIN, D), BF16), vm((H, WIN, D), BF16),
        vm(s_wq, BF16), vm(s_wo, BF16), vm(s_ckv, BF16),
        vm(s_bwq, BF16), vm(s_bwu, BF16), vm(s_bwu, BF16), vm(s_wo, BF16),
        vm((H, D), F32), vm((H, D), F32), vm((H, D), F32), vm((H, D), F32),
        vm((H, D), F32), vm((H, D), F32), vm((H, D), F32), vm((H, D), F32),
        vm((16, HD), BF16), vm((M, D), F32),
        vm((M * 8 + 8, D), F32), vm((D, C), BF16), vm((D, SK), F32), vm((C, D), F32),
        pltpu.SemaphoreType.DMA((5 + 2 * KV_GROUPS + 6,)),
        pltpu.SemaphoreType.DMA((10,)),
    ]
    any_spec = pl.BlockSpec(memory_space=pl.ANY)
    outs = pl.pallas_call(
        _kernel,
        out_shape=out_shape,
        in_specs=[any_spec] * 12,
        out_specs=(any_spec,) * 12,
        scratch_shapes=scratch,
        compiler_params=pltpu.CompilerParams(vmem_limit_bytes=120 * 1024 * 1024,
                                             disable_semaphore_checks=True),
        name="fused_decode_fwd_bwd",
    )(
        A_x,
        A_k_cache.reshape(H, SK, D),
        A_v_cache.reshape(H, SK, D),
        A_wq,
        A_wo,
        B_x,
        B_c_kv.reshape(SK, C),
        B_w_q.reshape(M * H, D),
        B_w_uk.reshape(C * H, D),
        B_w_uv.reshape(C * H, D),
        B_w_o.reshape(HD, M),
        grad_out,
    )
    (out, gax, gak, gav, gawq, gawo, gbx, gckv, gbwq, gbwuk, gbwuv, gbwo) = outs
    return (
        out,
        gax,
        gak.reshape(1, H, SK, D),
        gav.reshape(1, H, SK, D),
        gawq.reshape(M, HD),
        gawo.reshape(HD, M),
        gbx,
        gckv.reshape(1, SK, C),
        gbwq.reshape(M, H, D),
        gbwuk.reshape(C, H, D),
        gbwuv.reshape(C, H, D),
        gbwo.reshape(H, D, M),
    )
```

```python
import jax
import jax.numpy as jnp
from jax import lax
import jax.experimental.pallas as pl
import jax.experimental.pallas.tpu as pltpu

F32 = jnp.float32
BF16 = jnp.bfloat16

H = 32
D = 128
SK = 4096
WIN = 1024
M = 640
C = 512
HD = H * D
SCALE = float(D) ** -0.5

KV_GROUPS = 4
HPG = H // KV_GROUPS
CKV_SPLIT = 3072
NSEM = 2 + KV_GROUPS

ZR = 128
ZJ = 8
NZB = (SK - WIN) // ZR
NDB = WIN // ZR
NHG = H // ZJ
S_AWQ = (5, M // 5, HD)
S_WO = (8, HD // 8, M)
S_CKV = (8, SK // 8, C)
S_BWQ = (5, M * H // 5, D)
S_BWU = (8, C * H // 8, D)
AWQ_ROWS, AWQ_COLS = 8, 1024
WO_ROWS = 32
CKV_ROWS = 32
BWQ_ROWS = 64
BWU_ROWS = 64

NT = (((1,), (1,)), ((), ()))


def _dot(a, b):
    return jnp.dot(a, b, preferred_element_type=F32)


def _dot_nt(a, b):
    return lax.dot_general(a, b, NT, preferred_element_type=F32)


def _iota(shape, dim):
    return lax.broadcasted_iota(jnp.int32, shape, dim)


def _colrep(row):
    eye = _iota((128, 128), 0) == _iota((128, 128), 1)
    lhs = jnp.where(eye, jnp.broadcast_to(row, (128, 128)), 0.0).astype(BF16)
    return _dot(lhs, jnp.ones((128, 128), BF16))


def _kernel(
    ax_h, ak_h, av_h, awq_h, awo_h, bx_h, ckv_h, bwq_h, bwuk_h, bwuv_h, bwo_h, g_h,
    out_h, gax_h, gak_h, gav_h, gawq_h, gawo_h, gbx_h, gckv_h, gbwq_h, gbwuk_h, gbwuv_h, gbwo_h,
    ax_v, bx_v, g_v, k_v, v_v, awq_v, awo_v, ckv_v, bwq_v, bwuk_v, bwuv_v, bwo_v,
    out_s, gax_s, gbx_s, z_s, gk_s, gv_s, gawq_s, gawo_s, gckv_s, gbwq_s, gbwuk_s, gbwuv_s, gbwo_s,
    qa_s, doa_s, oa_s, dqa_s, qb_s, dctx_s, ctx_s, dqb_s, row_s, xrep_s, t_s, qd_s, ps_s, latt_s,
    sems,
):
    def rd(src, dst, k):
        return pltpu.make_async_copy(src, dst, sems.at[k])

    rd_first = [rd(awq_h, awq_v, 0), rd(ax_h, ax_v, 0), rd(bx_h, bx_v, 0), rd(g_h, g_v, 0)]
    rd_awo = rd(awo_h, awo_v, 1)
    rd_kv = []
    for gi in range(KV_GROUPS):
        hs = pl.ds(gi * HPG, HPG)
        rd_kv.append([rd(ak_h.at[hs, pl.ds(SK - WIN, WIN), :], k_v.at[hs], 2 + gi),
                      rd(av_h.at[hs, pl.ds(SK - WIN, WIN), :], v_v.at[hs], 2 + gi)])
    rd_bwq = rd(bwq_h, bwq_v, 0)
    rd_bwo = rd(bwo_h, bwo_v, 1)
    rd_bwuk = rd(bwuk_h, bwuk_v, 2)
    rd_bwuv = [rd(bwuv_h, bwuv_v, 3),
               rd(ckv_h.at[pl.ds(0, CKV_SPLIT)], ckv_v.at[pl.ds(0, CKV_SPLIT)], 3)]
    rd_ckv1 = rd(ckv_h.at[pl.ds(CKV_SPLIT, SK - CKV_SPLIT)],
                 ckv_v.at[pl.ds(CKV_SPLIT, SK - CKV_SPLIT)], 4)

    wsem = sems.at[0]

    def zero_copy(dst_h, i):
        h0 = (i // NZB) * ZJ
        r0 = pl.multiple_of((i % NZB) * ZR, ZR)
        return pltpu.make_async_copy(z_s, dst_h.at[pl.ds(h0, ZJ), pl.ds(r0, ZR), :], wsem)

    def cache_copy(src, dst_h, i):
        h0 = (i // NDB) * ZJ
        r0 = pl.multiple_of((i % NDB) * ZR, ZR)
        return pltpu.make_async_copy(
            src.at[pl.ds(h0, ZJ), pl.ds(r0, ZR), :],
            dst_h.at[pl.ds(h0, ZJ), pl.ds(pl.multiple_of(SK - WIN + r0, ZR), ZR), :], wsem)

    def rows_copy(src, dst_h, rows):
        def mk(i):
            r0 = pl.multiple_of(i * rows, rows)
            return pltpu.make_async_copy(src.at[:, pl.ds(r0, rows), :], dst_h.at[:, pl.ds(r0, rows), :], wsem)
        return mk, src.shape[1] // rows

    awq_nc = HD // AWQ_COLS

    def awq_copy(i):
        r0 = pl.multiple_of((i // awq_nc) * AWQ_ROWS, AWQ_ROWS)
        c0 = pl.multiple_of((i % awq_nc) * AWQ_COLS, AWQ_COLS)
        return pltpu.make_async_copy(gawq_s.at[:, pl.ds(r0, AWQ_ROWS), pl.ds(c0, AWQ_COLS)],
                                     gawq_h.at[:, pl.ds(r0, AWQ_ROWS), pl.ds(c0, AWQ_COLS)], wsem)

    writes = {
        "zk": (lambda i: zero_copy(gak_h, i), NHG * NZB),
        "zv": (lambda i: zero_copy(gav_h, i), NHG * NZB),
        "gk": (lambda i: cache_copy(gk_s, gak_h, i), NHG * NDB),
        "gv": (lambda i: cache_copy(gv_s, gav_h, i), NHG * NDB),
        "gckv": rows_copy(gckv_s, gckv_h, CKV_ROWS),
        "gbwuk": rows_copy(gbwuk_s, gbwuk_h, BWU_ROWS),
        "gbwuv": rows_copy(gbwuv_s, gbwuv_h, BWU_ROWS),
        "gbwo": rows_copy(gbwo_s, gbwo_h, WO_ROWS),
        "gbwq": rows_copy(gbwq_s, gbwq_h, BWQ_ROWS),
        "gawo": rows_copy(gawo_s, gawo_h, WO_ROWS),
        "gawq": (awq_copy, (S_AWQ[1] // AWQ_ROWS) * awq_nc),
    }
    small_writes = [
        pltpu.make_async_copy(out_s, out_h, wsem),
        pltpu.make_async_copy(gax_s, gax_h, wsem),
        pltpu.make_async_copy(gbx_s, gbx_h, wsem),
    ]
    issued = {name: 0 for name in writes}

    def issue(name, count=None):
        mk, n = writes[name]
        lo = issued[name]
        hi = n if count is None else lo + count
        assert lo < hi <= n
        issued[name] = hi

        def body(i, carry):
            mk(i).start()
            return carry
        lax.fori_loop(lo, hi, body, 0)

    def wait_writes(name):
        mk, n = writes[name]
        assert issued[name] == n

        def body(i, carry):
            mk(i).wait()
            return carry
        lax.fori_loop(0, n, body, 0)

    def xa():
        return ax_v[0].astype(F32)

    def xb():
        return bx_v[0].astype(F32)

    def ga():
        return g_v[0][:, :M].astype(F32)

    def gb():
        return g_v[0][:, M:].astype(F32)

    def put_rows(dst, r, n, val, cols=slice(None)):
        rps = dst.shape[1]
        dst[r // rps, pl.ds(pl.multiple_of(r % rps, n), n), cols] = val

    def rows16(row):
        return jnp.broadcast_to(row, (16, row.shape[1])).astype(BF16)

    def row_to_heads(row, dst):
        for h in range(H):
            dst[h:h + 1, :] = row[0:1, h * D:(h + 1) * D]

    def heads_to_row(src):
        for h in range(H):
            row_s[:, h * D:(h + 1) * D] = jnp.broadcast_to(src[h:h + 1, :], (16, D)).astype(BF16)
        return row_s[...]

    def fill_xrep(x):
        for t in range(M // 128):
            xrep_s[t * 128:(t + 1) * 128, :] = _colrep(x[:, t * 128:(t + 1) * 128])

    def outer_wo(src, grow, dst):
        def body(h, carry):
            col = _colrep(src[pl.ds(h, 1), :])
            for t in range(M // 128):
                cols = slice(t * 128, (t + 1) * 128)
                put_rows(dst, h * D, D, (col * grow[:, cols]).astype(BF16), cols)
            return carry
        lax.fori_loop(0, H, body, 0)

    def a_q():
        row_to_heads(_dot(rows16(xa()), awq_v[...]), qa_s)

    def a_do():
        row_to_heads(_dot_nt(rows16(ga()), awo_v[...]), doa_s)

    def a_head(h, carry):
        kk = k_v[h]
        vv = v_v[h]
        q = qa_s[pl.ds(h, 1), :]
        do = doa_s[pl.ds(h, 1), :]
        s = _dot_nt(kk, jnp.broadcast_to(q, (D, D)).astype(BF16)) * SCALE
        dp = _dot_nt(vv, jnp.broadcast_to(do, (D, D)).astype(BF16))
        e = jnp.exp(s - jnp.max(s, axis=0, keepdims=True))
        inv = 1.0 / jnp.sum(e, axis=0, keepdims=True)
        u = e * (dp - jnp.sum(e * dp, axis=0, keepdims=True) * inv)
        f = inv * SCALE
        gk_s[h] = (u * (q * f)).astype(BF16)
        gv_s[h] = (e * (do * inv)).astype(BF16)
        oa_s[pl.ds(h, 1), :] = jnp.sum(e * vv.astype(F32), axis=0, keepdims=True) * inv
        dqa_s[pl.ds(h, 1), :] = jnp.sum(u * kk.astype(F32), axis=0, keepdims=True) * f
        return carry

    def a_out():
        out_s[0, :, 0:M] = _dot(heads_to_row(oa_s), awo_v[...])[0:1].astype(BF16)

    def a_dwo():
        outer_wo(oa_s, ga(), gawo_s)

    def a_dx():
        gax_s[0] = _dot_nt(heads_to_row(dqa_s), awq_v[...])[0:1].astype(BF16)

    def a_dwq():
        fill_xrep(xa())
        for h in range(H):
            blk = (xrep_s[...] * dqa_s[h:h + 1, :]).astype(BF16)
            gawq_s[:, :, h * D:(h + 1) * D] = blk.reshape(S_AWQ[0], S_AWQ[1], D)

    def b_q():
        fill_xrep(xb())

        def body(i, acc):
            for j in range(8):
                m = i * 8 + j
                w = bwq_v[pl.ds(pl.multiple_of(m * H, H), H), :].astype(F32)
                acc = acc + w * xrep_s[pl.ds(m, 1), :]
            return acc
        qb_s[...] = lax.fori_loop(0, M // 8, body, jnp.zeros((H, D), F32))

    def b_dctx():
        row_to_heads(_dot_nt(rows16(gb()), bwo_v[...]), dctx_s)

    def b_absorb(w_v, vec_s, first):
        cb = 16
        diag = (_iota((cb * H, D), 0) % H) == (_iota((cb * H, D), 1) % H)
        zpad = jnp.zeros((H, D), F32)
        parts = [vec_s[...], zpad, zpad, zpad] if first else [zpad, vec_s[...], zpad, zpad]
        rhs = jnp.concatenate(parts, axis=0).astype(BF16)

        def body(i, carry):
            r0 = pl.multiple_of(i * cb * H, cb * H)
            r = _dot_nt(w_v[pl.ds(r0, cb * H), :], rhs)
            r = jnp.sum(jnp.where(diag, r, 0.0).reshape(cb, H, D), axis=1)
            t0 = pl.multiple_of(i * cb, cb)
            if first:
                t_s[pl.ds(t0, cb), :] = r
            else:
                t_s[pl.ds(t0, cb), :] = t_s[pl.ds(t0, cb), :] + r
            return carry
        lax.fori_loop(0, C // cb, body, 0)

    def b_qd():
        qd_s[...] = t_s[0:C, :].T.astype(BF16)

    def b_attn():
        sd = _dot_nt(qd_s[0:2 * H, :], ckv_v[...])
        s = sd[0:H] * SCALE
        dp = sd[H:2 * H]
        e = jnp.exp(s - jnp.max(s, axis=1, keepdims=True))
        p = e * (1.0 / jnp.sum(e, axis=1, keepdims=True))
        ds = p * (dp - jnp.sum(p * dp, axis=1, keepdims=True)) * SCALE
        ps_s[0:H, :] = ds
        ps_s[H:2 * H, :] = p
        ps_s[2 * H:4 * H, :] = jnp.zeros((2 * H, SK), F32)
        lat = _dot(ps_s[...].astype(BF16), ckv_v[...])
        latt_s[...] = lat.T

    def b_dckv():
        def body(j, carry):
            k0 = pl.multiple_of(j * 512, 512)
            pst = ps_s[:, pl.ds(k0, 512)].T.astype(BF16)
            put_rows(gckv_s, j * 512, 512, _dot(pst, qd_s[...]).astype(BF16))
            return carry
        lax.fori_loop(0, SK // 512, body, 0)

    def b_lat():
        cc = 8
        sel = (_iota((cc * H, D), 0) % H) == (_iota((cc * H, D), 1) % H)
        jj = _iota((D, 2 * D), 0)
        nn = _iota((D, 2 * D), 1)
        expand = jnp.where(((jj < H) & (nn < D)) | ((jj >= H) & (jj < 2 * H) & (nn >= D)), 1.0, 0.0).astype(BF16)
        qb_t = jnp.concatenate([qb_s[...]] * cc, axis=0)
        dctx_t = jnp.concatenate([dctx_s[...]] * cc, axis=0)

        def body(i, carry):
            dq_acc, ctx_acc = carry
            c0 = i * cc
            lhs = jnp.concatenate(
                [jnp.broadcast_to(latt_s[pl.ds(c0 + j, 1), :], (H, D)) for j in range(cc)], axis=0)
            rep = _dot(jnp.where(sel, lhs, 0.0).astype(BF16), expand)
            rep_ds = rep[:, 0:D]
            rep_p = rep[:, D:2 * D]
            put_rows(gbwuk_s, c0 * H, cc * H, (rep_ds * qb_t).astype(BF16))
            put_rows(gbwuv_s, c0 * H, cc * H, (rep_p * dctx_t).astype(BF16))
            r0 = pl.multiple_of(c0 * H, cc * H)
            wk = bwuk_v[pl.ds(r0, cc * H), :].astype(F32)
            wv = bwuv_v[pl.ds(r0, cc * H), :].astype(F32)
            dq_acc = dq_acc + jnp.sum((rep_ds * wk).reshape(cc, H, D), axis=0)
            ctx_acc = ctx_acc + jnp.sum((rep_p * wv).reshape(cc, H, D), axis=0)
            return dq_acc, ctx_acc

        dqb, ctx = lax.fori_loop(0, C // cc, body, (jnp.zeros((H, D), F32), jnp.zeros((H, D), F32)))
        ctx_s[...] = ctx
        dqb_s[...] = dqb

    def b_out():
        out_s[0, :, M:2 * M] = _dot(heads_to_row(ctx_s), bwo_v[...])[0:1].astype(BF16)

    def b_dwo():
        outer_wo(ctx_s, gb(), gbwo_s)

    def b_dwq():
        def body(i, carry):
            dq = dqb_s[...]
            for j in range(8):
                m = i * 8 + j
                w = bwq_v[pl.ds(pl.multiple_of(m * H, H), H), :].astype(F32) * dq
                t_s[pl.ds(m, 1), :] = jnp.sum(w, axis=0, keepdims=True)
                put_rows(gbwq_s, m * H, H, (xrep_s[pl.ds(m, 1), :] * dq).astype(BF16))
            return carry
        lax.fori_loop(0, M // 8, body, 0)
        gbx_s[0] = jnp.sum(t_s[...].T, axis=0, keepdims=True).astype(BF16)

    for cp in rd_first:
        cp.start()
    rd_awo.start()
    for pair in rd_kv:
        for cp in pair:
            cp.start()
    z_s[...] = jnp.zeros(z_s.shape, BF16)

    for cp in rd_first:
        cp.wait()
    rd_bwq.start()
    a_q()
    rd_awo.wait()
    rd_bwo.start()
    a_do()
    for gi in range(KV_GROUPS):
        for cp in rd_kv[gi]:
            cp.wait()
        if gi == 0:
            rd_bwuk.start()
        elif gi == 1:
            for cp in rd_bwuv:
                cp.start()
        elif gi == 2:
            rd_ckv1.start()
        lax.fori_loop(gi * HPG, (gi + 1) * HPG, a_head, 0)
    rd_bwq.wait()
    b_q()
    rd_bwo.wait()
    b_dctx()
    rd_bwuk.wait()
    for cp in rd_bwuv:
        cp.wait()

    issue("zk", 72)
    b_absorb(bwuk_v, qb_s, True)
    issue("zk", 18)
    b_absorb(bwuv_v, dctx_s, False)
    b_qd()
    issue("zk")
    issue("zv", 14)
    rd_ckv1.wait()
    b_attn()
    issue("zv", 14)
    b_dckv()
    issue("zv", 14)
    b_lat()
    issue("zv", 36)
    b_out()
    b_dwo()
    issue("zv")
    b_dwq()
    issue("gk", 16)
    a_out()
    a_dwo()
    issue("gk")
    a_dx()
    a_dwq()
    for cp in small_writes:
        cp.start()
    rest = ("gv", "gckv", "gbwuk", "gbwuv", "gbwo", "gbwq", "gawo", "gawq")
    for name in rest:
        issue(name)

    for name in ("zk", "zv", "gk"):
        wait_writes(name)
    for cp in small_writes:
        cp.wait()
    for name in rest:
        wait_writes(name)


@jax.jit
def pallas_concat_heads__sliding_block_cached__compressed_kv_cla__decode_kernel(
    A_x: jax.Array,
    A_k_cache: jax.Array,
    A_v_cache: jax.Array,
    A_wq: jax.Array,
    A_wo: jax.Array,
    B_x: jax.Array,
    B_c_kv: jax.Array,
    B_w_q: jax.Array,
    B_w_uk: jax.Array,
    B_w_uv: jax.Array,
    B_w_o: jax.Array,
    grad_out: jax.Array,
):
    sds = jax.ShapeDtypeStruct
    out_shape = (
        sds((1, 1, 2 * M), BF16),
        sds((1, 1, M), BF16),
        sds((H, SK, D), BF16),
        sds((H, SK, D), BF16),
        sds(S_AWQ, BF16),
        sds(S_WO, BF16),
        sds((1, 1, M), BF16),
        sds(S_CKV, BF16),
        sds(S_BWQ, BF16),
        sds(S_BWU, BF16),
        sds(S_BWU, BF16),
        sds(S_WO, BF16),
    )
    vm = pltpu.VMEM
    scratch = [
        vm((1, 1, M), BF16), vm((1, 1, M), BF16), vm((1, 1, 2 * M), BF16),
        vm((H, WIN, D), BF16), vm((H, WIN, D), BF16),
        vm((M, HD), BF16), vm((HD, M), BF16),
        vm((SK, C), BF16),
        vm((M * H, D), BF16), vm((C * H, D), BF16), vm((C * H, D), BF16), vm((HD, M), BF16),
        vm((1, 1, 2 * M), BF16), vm((1, 1, M), BF16), vm((1, 1, M), BF16),
        vm((ZJ, ZR, D), BF16),
        vm((H, WIN, D), BF16), vm((H, WIN, D), BF16),
        vm(S_AWQ, BF16), vm(S_WO, BF16), vm(S_CKV, BF16),
        vm(S_BWQ, BF16), vm(S_BWU, BF16), vm(S_BWU, BF16), vm(S_WO, BF16),
        vm((H, D), F32), vm((H, D), F32), vm((H, D), F32), vm((H, D), F32),
        vm((H, D), F32), vm((H, D), F32), vm((H, D), F32), vm((H, D), F32),
        vm((16, HD), BF16), vm((M, D), F32),
        vm((M, D), F32), vm((D, C), BF16), vm((D, SK), F32), vm((C, D), F32),
        pltpu.SemaphoreType.DMA((NSEM,)),
    ]
    any_spec = pl.BlockSpec(memory_space=pl.ANY)
    outs = pl.pallas_call(
        _kernel,
        out_shape=out_shape,
        in_specs=[any_spec] * 12,
        out_specs=(any_spec,) * 12,
        scratch_shapes=scratch,
        compiler_params=pltpu.CompilerParams(vmem_limit_bytes=120 * 1024 * 1024),
        name="fused_decode_fwd_bwd",
    )(
        A_x,
        A_k_cache.reshape(H, SK, D),
        A_v_cache.reshape(H, SK, D),
        A_wq,
        A_wo,
        B_x,
        B_c_kv.reshape(SK, C),
        B_w_q.reshape(M * H, D),
        B_w_uk.reshape(C * H, D),
        B_w_uv.reshape(C * H, D),
        B_w_o.reshape(HD, M),
        grad_out,
    )
    (out, gax, gak, gav, gawq, gawo, gbx, gckv, gbwq, gbwuk, gbwuv, gbwo) = outs
    return (
        out,
        gax,
        gak.reshape(1, H, SK, D),
        gav.reshape(1, H, SK, D),
        gawq.reshape(M, HD),
        gawo.reshape(HD, M),
        gbx,
        gckv.reshape(1, SK, C),
        gbwq.reshape(M, H, D),
        gbwuk.reshape(C, H, D),
        gbwuv.reshape(C, H, D),
        gbwo.reshape(H, D, M),
    )
```

```python
import jax
import jax.numpy as jnp
from jax import lax
import jax.experimental.pallas as pl
import jax.experimental.pallas.tpu as pltpu

F32 = jnp.float32
BF16 = jnp.bfloat16

H = 32
D = 128
SK = 4096
WIN = 1024
M = 640
C = 512
HD = H * D
SCALE = float(D) ** -0.5

KV_GROUPS = 4
HPG = H // KV_GROUPS
CKV_SPLIT = 3072
NSEM = 2 + KV_GROUPS

ZR = 128
ZJ = 8
NZB = (SK - WIN) // ZR
NDB = WIN // ZR
NHG = H // ZJ
S_AWQ = (5, M // 5, HD)
S_WO = (8, HD // 8, M)
S_CKV = (8, SK // 8, C)
S_BWQ = (5, M * H // 5, D)
S_BWU = (8, C * H // 8, D)
AWQ_ROWS, AWQ_COLS = 8, 1024
WO_ROWS = 32
CKV_ROWS = 32
BWQ_ROWS = 64
BWU_ROWS = 64

NT = (((1,), (1,)), ((), ()))


def _dot(a, b):
    return jnp.dot(a, b, preferred_element_type=F32)


def _dot_nt(a, b):
    return lax.dot_general(a, b, NT, preferred_element_type=F32)


def _iota(shape, dim):
    return lax.broadcasted_iota(jnp.int32, shape, dim)


def _colrep(row):
    eye = _iota((128, 128), 0) == _iota((128, 128), 1)
    lhs = jnp.where(eye, jnp.broadcast_to(row, (128, 128)), 0.0).astype(BF16)
    return _dot(lhs, jnp.ones((128, 128), BF16))


def _kernel(
    ax_h, ak_h, av_h, awq_h, awo_h, bx_h, ckv_h, bwq_h, bwuk_h, bwuv_h, bwo_h, g_h,
    out_h, gax_h, gak_h, gav_h, gawq_h, gawo_h, gbx_h, gckv_h, gbwq_h, gbwuk_h, gbwuv_h, gbwo_h,
    ax_v, bx_v, g_v, k_v, v_v, awq_v, awo_v, ckv_v, bwq_v, bwuk_v, bwuv_v, bwo_v,
    out_s, gax_s, gbx_s, z_s, gk_s, gv_s, gawq_s, gawo_s, gckv_s, gbwq_s, gbwuk_s, gbwuv_s, gbwo_s,
    qa_s, doa_s, oa_s, dqa_s, qb_s, dctx_s, ctx_s, dqb_s, row_s, xrep_s, t_s, qd_s, ps_s, latt_s,
    sems,
):
    def rd(src, dst, k):
        return pltpu.make_async_copy(src, dst, sems.at[k])

    rd_first = [rd(awq_h, awq_v, 0), rd(ax_h, ax_v, 0), rd(bx_h, bx_v, 0), rd(g_h, g_v, 0)]
    rd_awo = rd(awo_h, awo_v, 1)
    rd_kv = []
    for gi in range(KV_GROUPS):
        hs = pl.ds(gi * HPG, HPG)
        rd_kv.append([rd(ak_h.at[hs, pl.ds(SK - WIN, WIN), :], k_v.at[hs], 2 + gi),
                      rd(av_h.at[hs, pl.ds(SK - WIN, WIN), :], v_v.at[hs], 2 + gi)])
    rd_bwq = rd(bwq_h, bwq_v, 0)
    rd_bwo = rd(bwo_h, bwo_v, 1)
    rd_bwuk = rd(bwuk_h, bwuk_v, 2)
    rd_bwuv = [rd(bwuv_h, bwuv_v, 3),
               rd(ckv_h.at[pl.ds(0, CKV_SPLIT)], ckv_v.at[pl.ds(0, CKV_SPLIT)], 3)]
    rd_ckv1 = rd(ckv_h.at[pl.ds(CKV_SPLIT, SK - CKV_SPLIT)],
                 ckv_v.at[pl.ds(CKV_SPLIT, SK - CKV_SPLIT)], 4)

    wsem = sems.at[0]

    def zero_copy(dst_h, i):
        h0 = (i // NZB) * ZJ
        r0 = pl.multiple_of((i % NZB) * ZR, ZR)
        return pltpu.make_async_copy(z_s, dst_h.at[pl.ds(h0, ZJ), pl.ds(r0, ZR), :], wsem)

    def cache_copy(src, dst_h, i):
        h0 = (i // NDB) * ZJ
        r0 = pl.multiple_of((i % NDB) * ZR, ZR)
        return pltpu.make_async_copy(
            src.at[pl.ds(h0, ZJ), pl.ds(r0, ZR), :],
            dst_h.at[pl.ds(h0, ZJ), pl.ds(pl.multiple_of(SK - WIN + r0, ZR), ZR), :], wsem)

    def rows_copy(src, dst_h, rows):
        def mk(i):
            r0 = pl.multiple_of(i * rows, rows)
            return pltpu.make_async_copy(src.at[:, pl.ds(r0, rows), :], dst_h.at[:, pl.ds(r0, rows), :], wsem)
        return mk, src.shape[1] // rows

    awq_nc = HD // AWQ_COLS

    def awq_copy(i):
        r0 = pl.multiple_of((i // awq_nc) * AWQ_ROWS, AWQ_ROWS)
        c0 = pl.multiple_of((i % awq_nc) * AWQ_COLS, AWQ_COLS)
        return pltpu.make_async_copy(gawq_s.at[:, pl.ds(r0, AWQ_ROWS), pl.ds(c0, AWQ_COLS)],
                                     gawq_h.at[:, pl.ds(r0, AWQ_ROWS), pl.ds(c0, AWQ_COLS)], wsem)

    writes = {
        "zk": (lambda i: zero_copy(gak_h, i), NHG * NZB),
        "zv": (lambda i: zero_copy(gav_h, i), NHG * NZB),
        "gk": (lambda i: cache_copy(gk_s, gak_h, i), NHG * NDB),
        "gv": (lambda i: cache_copy(gv_s, gav_h, i), NHG * NDB),
        "gckv": rows_copy(gckv_s, gckv_h, CKV_ROWS),
        "gbwuk": rows_copy(gbwuk_s, gbwuk_h, BWU_ROWS),
        "gbwuv": rows_copy(gbwuv_s, gbwuv_h, BWU_ROWS),
        "gbwo": rows_copy(gbwo_s, gbwo_h, WO_ROWS),
        "gbwq": rows_copy(gbwq_s, gbwq_h, BWQ_ROWS),
        "gawo": rows_copy(gawo_s, gawo_h, WO_ROWS),
        "gawq": (awq_copy, (S_AWQ[1] // AWQ_ROWS) * awq_nc),
    }
    small_writes = [
        pltpu.make_async_copy(out_s, out_h, wsem),
        pltpu.make_async_copy(gax_s, gax_h, wsem),
        pltpu.make_async_copy(gbx_s, gbx_h, wsem),
    ]
    issued = {name: 0 for name in writes}

    def issue(name, count=None):
        mk, n = writes[name]
        lo = issued[name]
        hi = n if count is None else lo + count
        assert lo < hi <= n
        issued[name] = hi

        def body(i, carry):
            mk(i).start()
            return carry
        lax.fori_loop(lo, hi, body, 0)

    early = ("zk", "zv", "gk", "gv")

    def top_up(count):
        for name in early:
            k = min(count, writes[name][1] - issued[name])
            if k > 0:
                issue(name, k)
                count -= k

    def wait_writes(name):
        mk, n = writes[name]
        assert issued[name] == n

        def body(i, carry):
            mk(i).wait()
            return carry
        lax.fori_loop(0, n, body, 0)

    def xa():
        return ax_v[0].astype(F32)

    def xb():
        return bx_v[0].astype(F32)

    def ga():
        return g_v[0][:, :M].astype(F32)

    def gb():
        return g_v[0][:, M:].astype(F32)

    def put_rows(dst, r, n, val, cols=slice(None)):
        rps = dst.shape[1]
        dst[r // rps, pl.ds(pl.multiple_of(r % rps, n), n), cols] = val

    def rows16(row):
        return jnp.broadcast_to(row, (16, row.shape[1])).astype(BF16)

    def row_to_heads(row, dst):
        for h in range(H):
            dst[h:h + 1, :] = row[0:1, h * D:(h + 1) * D]

    def heads_to_row(src):
        for h in range(H):
            row_s[:, h * D:(h + 1) * D] = jnp.broadcast_to(src[h:h + 1, :], (16, D)).astype(BF16)
        return row_s[...]

    def fill_xrep(x):
        for t in range(M // 128):
            xrep_s[t * 128:(t + 1) * 128, :] = _colrep(x[:, t * 128:(t + 1) * 128])

    def outer_wo(src, grow, dst):
        def body(h, carry):
            col = _colrep(src[pl.ds(h, 1), :])
            for t in range(M // 128):
                cols = slice(t * 128, (t + 1) * 128)
                put_rows(dst, h * D, D, (col * grow[:, cols]).astype(BF16), cols)
            return carry
        lax.fori_loop(0, H, body, 0)

    def a_q():
        row_to_heads(_dot(rows16(xa()), awq_v[...]), qa_s)

    def a_do():
        row_to_heads(_dot_nt(rows16(ga()), awo_v[...]), doa_s)

    def a_head(h, carry):
        kk = k_v[h]
        vv = v_v[h]
        q = qa_s[pl.ds(h, 1), :]
        do = doa_s[pl.ds(h, 1), :]
        s = _dot_nt(kk, jnp.broadcast_to(q, (D, D)).astype(BF16)) * SCALE
        dp = _dot_nt(vv, jnp.broadcast_to(do, (D, D)).astype(BF16))
        e = jnp.exp(s - jnp.max(s, axis=0, keepdims=True))
        inv = 1.0 / jnp.sum(e, axis=0, keepdims=True)
        u = e * (dp - jnp.sum(e * dp, axis=0, keepdims=True) * inv)
        f = inv * SCALE
        gk_s[h] = (u * (q * f)).astype(BF16)
        gv_s[h] = (e * (do * inv)).astype(BF16)
        oa_s[pl.ds(h, 1), :] = jnp.sum(e * vv.astype(F32), axis=0, keepdims=True) * inv
        dqa_s[pl.ds(h, 1), :] = jnp.sum(u * kk.astype(F32), axis=0, keepdims=True) * f
        return carry

    def a_out():
        out_s[0, :, 0:M] = _dot(heads_to_row(oa_s), awo_v[...])[0:1].astype(BF16)

    def a_dwo():
        outer_wo(oa_s, ga(), gawo_s)

    def a_dx():
        gax_s[0] = _dot_nt(heads_to_row(dqa_s), awq_v[...])[0:1].astype(BF16)

    def a_dwq():
        fill_xrep(xa())
        for h in range(H):
            blk = (xrep_s[...] * dqa_s[h:h + 1, :]).astype(BF16)
            gawq_s[:, :, h * D:(h + 1) * D] = blk.reshape(S_AWQ[0], S_AWQ[1], D)

    def b_q():
        fill_xrep(xb())

        def body(i, acc):
            for j in range(8):
                m = i * 8 + j
                w = bwq_v[pl.ds(pl.multiple_of(m * H, H), H), :].astype(F32)
                acc = acc + w * xrep_s[pl.ds(m, 1), :]
            return acc
        qb_s[...] = lax.fori_loop(0, M // 8, body, jnp.zeros((H, D), F32))

    def b_dctx():
        row_to_heads(_dot_nt(rows16(gb()), bwo_v[...]), dctx_s)

    def b_absorb(w_v, vec_s, first):
        cb = 16
        diag = (_iota((cb * H, D), 0) % H) == (_iota((cb * H, D), 1) % H)
        zpad = jnp.zeros((H, D), F32)
        parts = [vec_s[...], zpad, zpad, zpad] if first else [zpad, vec_s[...], zpad, zpad]
        rhs = jnp.concatenate(parts, axis=0).astype(BF16)

        def body(i, carry):
            r0 = pl.multiple_of(i * cb * H, cb * H)
            r = _dot_nt(w_v[pl.ds(r0, cb * H), :], rhs)
            r = jnp.sum(jnp.where(diag, r, 0.0).reshape(cb, H, D), axis=1)
            t0 = pl.multiple_of(i * cb, cb)
            if first:
                t_s[pl.ds(t0, cb), :] = r
            else:
                t_s[pl.ds(t0, cb), :] = t_s[pl.ds(t0, cb), :] + r
            return carry
        lax.fori_loop(0, C // cb, body, 0)

    def b_qd():
        qd_s[...] = t_s[0:C, :].T.astype(BF16)

    def b_attn():
        sd = _dot_nt(qd_s[0:2 * H, :], ckv_v[...])
        s = sd[0:H] * SCALE
        dp = sd[H:2 * H]
        e = jnp.exp(s - jnp.max(s, axis=1, keepdims=True))
        p = e * (1.0 / jnp.sum(e, axis=1, keepdims=True))
        ds = p * (dp - jnp.sum(p * dp, axis=1, keepdims=True)) * SCALE
        ps_s[0:H, :] = ds
        ps_s[H:2 * H, :] = p
        ps_s[2 * H:4 * H, :] = jnp.zeros((2 * H, SK), F32)
        lat = _dot(ps_s[...].astype(BF16), ckv_v[...])
        latt_s[...] = lat.T

    def b_dckv():
        def body(j, carry):
            k0 = pl.multiple_of(j * 512, 512)
            pst = ps_s[:, pl.ds(k0, 512)].T.astype(BF16)
            put_rows(gckv_s, j * 512, 512, _dot(pst, qd_s[...]).astype(BF16))
            return carry
        lax.fori_loop(0, SK // 512, body, 0)

    def b_lat():
        cc = 8
        sel = (_iota((cc * H, D), 0) % H) == (_iota((cc * H, D), 1) % H)
        jj = _iota((D, 2 * D), 0)
        nn = _iota((D, 2 * D), 1)
        expand = jnp.where(((jj < H) & (nn < D)) | ((jj >= H) & (jj < 2 * H) & (nn >= D)), 1.0, 0.0).astype(BF16)
        qb_t = jnp.concatenate([qb_s[...]] * cc, axis=0)
        dctx_t = jnp.concatenate([dctx_s[...]] * cc, axis=0)

        def body(i, carry):
            dq_acc, ctx_acc = carry
            c0 = i * cc
            lhs = jnp.concatenate(
                [jnp.broadcast_to(latt_s[pl.ds(c0 + j, 1), :], (H, D)) for j in range(cc)], axis=0)
            rep = _dot(jnp.where(sel, lhs, 0.0).astype(BF16), expand)
            rep_ds = rep[:, 0:D]
            rep_p = rep[:, D:2 * D]
            put_rows(gbwuk_s, c0 * H, cc * H, (rep_ds * qb_t).astype(BF16))
            put_rows(gbwuv_s, c0 * H, cc * H, (rep_p * dctx_t).astype(BF16))
            r0 = pl.multiple_of(c0 * H, cc * H)
            wk = bwuk_v[pl.ds(r0, cc * H), :].astype(F32)
            wv = bwuv_v[pl.ds(r0, cc * H), :].astype(F32)
            dq_acc = dq_acc + jnp.sum((rep_ds * wk).reshape(cc, H, D), axis=0)
            ctx_acc = ctx_acc + jnp.sum((rep_p * wv).reshape(cc, H, D), axis=0)
            return dq_acc, ctx_acc

        dqb, ctx = lax.fori_loop(0, C // cc, body, (jnp.zeros((H, D), F32), jnp.zeros((H, D), F32)))
        ctx_s[...] = ctx
        dqb_s[...] = dqb

    def b_out():
        out_s[0, :, M:2 * M] = _dot(heads_to_row(ctx_s), bwo_v[...])[0:1].astype(BF16)

    def b_dwo():
        outer_wo(ctx_s, gb(), gbwo_s)

    def b_dwq():
        def body(i, carry):
            dq = dqb_s[...]
            for j in range(8):
                m = i * 8 + j
                w = bwq_v[pl.ds(pl.multiple_of(m * H, H), H), :].astype(F32) * dq
                t_s[pl.ds(m, 1), :] = jnp.sum(w, axis=0, keepdims=True)
                put_rows(gbwq_s, m * H, H, (xrep_s[pl.ds(m, 1), :] * dq).astype(BF16))
            return carry
        lax.fori_loop(0, M // 8, body, 0)
        gbx_s[0] = jnp.sum(t_s[...].T, axis=0, keepdims=True).astype(BF16)

    for cp in rd_first:
        cp.start()
    rd_awo.start()
    for pair in rd_kv:
        for cp in pair:
            cp.start()
    z_s[...] = jnp.zeros(z_s.shape, BF16)

    for cp in rd_first:
        cp.wait()
    rd_bwq.start()
    a_q()
    rd_awo.wait()
    rd_bwo.start()
    a_do()
    for gi in range(KV_GROUPS):
        for cp in rd_kv[gi]:
            cp.wait()
        if gi == 0:
            rd_bwuk.start()
        elif gi == 1:
            for cp in rd_bwuv:
                cp.start()
        elif gi == 2:
            rd_ckv1.start()
        lax.fori_loop(gi * HPG, (gi + 1) * HPG, a_head, 0)
    rd_bwq.wait()
    rd_bwo.wait()
    rd_bwuk.wait()
    for cp in rd_bwuv:
        cp.wait()

    top_up(72)
    b_q()
    b_dctx()
    top_up(12)
    b_absorb(bwuk_v, qb_s, True)
    top_up(18)
    b_absorb(bwuv_v, dctx_s, False)
    b_qd()
    top_up(19)
    rd_ckv1.wait()
    b_attn()
    top_up(14)
    b_dckv()
    top_up(13)
    b_lat()
    top_up(35)
    b_out()
    b_dwo()
    top_up(18)
    b_dwq()
    top_up(16)
    a_out()
    a_dwo()
    top_up(18)
    a_dx()
    a_dwq()
    top_up(H * SK)
    for cp in small_writes:
        cp.start()
    late = ("gckv", "gbwuk", "gbwuv", "gbwo", "gbwq", "gawo", "gawq")
    for name in late:
        issue(name)

    for name in early:
        wait_writes(name)
    for cp in small_writes:
        cp.wait()
    for name in late:
        wait_writes(name)


@jax.jit
def pallas_concat_heads__sliding_block_cached__compressed_kv_cla__decode_kernel(
    A_x: jax.Array,
    A_k_cache: jax.Array,
    A_v_cache: jax.Array,
    A_wq: jax.Array,
    A_wo: jax.Array,
    B_x: jax.Array,
    B_c_kv: jax.Array,
    B_w_q: jax.Array,
    B_w_uk: jax.Array,
    B_w_uv: jax.Array,
    B_w_o: jax.Array,
    grad_out: jax.Array,
):
    sds = jax.ShapeDtypeStruct
    out_shape = (
        sds((1, 1, 2 * M), BF16),
        sds((1, 1, M), BF16),
        sds((H, SK, D), BF16),
        sds((H, SK, D), BF16),
        sds(S_AWQ, BF16),
        sds(S_WO, BF16),
        sds((1, 1, M), BF16),
        sds(S_CKV, BF16),
        sds(S_BWQ, BF16),
        sds(S_BWU, BF16),
        sds(S_BWU, BF16),
        sds(S_WO, BF16),
    )
    vm = pltpu.VMEM
    scratch = [
        vm((1, 1, M), BF16), vm((1, 1, M), BF16), vm((1, 1, 2 * M), BF16),
        vm((H, WIN, D), BF16), vm((H, WIN, D), BF16),
        vm((M, HD), BF16), vm((HD, M), BF16),
        vm((SK, C), BF16),
        vm((M * H, D), BF16), vm((C * H, D), BF16), vm((C * H, D), BF16), vm((HD, M), BF16),
        vm((1, 1, 2 * M), BF16), vm((1, 1, M), BF16), vm((1, 1, M), BF16),
        vm((ZJ, ZR, D), BF16),
        vm((H, WIN, D), BF16), vm((H, WIN, D), BF16),
        vm(S_AWQ, BF16), vm(S_WO, BF16), vm(S_CKV, BF16),
        vm(S_BWQ, BF16), vm(S_BWU, BF16), vm(S_BWU, BF16), vm(S_WO, BF16),
        vm((H, D), F32), vm((H, D), F32), vm((H, D), F32), vm((H, D), F32),
        vm((H, D), F32), vm((H, D), F32), vm((H, D), F32), vm((H, D), F32),
        vm((16, HD), BF16), vm((M, D), F32),
        vm((M, D), F32), vm((D, C), BF16), vm((D, SK), F32), vm((C, D), F32),
        pltpu.SemaphoreType.DMA((NSEM,)),
    ]
    any_spec = pl.BlockSpec(memory_space=pl.ANY)
    outs = pl.pallas_call(
        _kernel,
        out_shape=out_shape,
        in_specs=[any_spec] * 12,
        out_specs=(any_spec,) * 12,
        scratch_shapes=scratch,
        compiler_params=pltpu.CompilerParams(vmem_limit_bytes=120 * 1024 * 1024),
        name="fused_decode_fwd_bwd",
    )(
        A_x,
        A_k_cache.reshape(H, SK, D),
        A_v_cache.reshape(H, SK, D),
        A_wq,
        A_wo,
        B_x,
        B_c_kv.reshape(SK, C),
        B_w_q.reshape(M * H, D),
        B_w_uk.reshape(C * H, D),
        B_w_uv.reshape(C * H, D),
        B_w_o.reshape(HD, M),
        grad_out,
    )
    (out, gax, gak, gav, gawq, gawo, gbx, gckv, gbwq, gbwuk, gbwuv, gbwo) = outs
    return (
        out,
        gax,
        gak.reshape(1, H, SK, D),
        gav.reshape(1, H, SK, D),
        gawq.reshape(M, HD),
        gawo.reshape(HD, M),
        gbx,
        gckv.reshape(1, SK, C),
        gbwq.reshape(M, H, D),
        gbwuk.reshape(C, H, D),
        gbwuv.reshape(C, H, D),
        gbwo.reshape(H, D, M),
    )
```

```python
import jax
import jax.numpy as jnp
from jax import lax
import jax.experimental.pallas as pl
import jax.experimental.pallas.tpu as pltpu

F32 = jnp.float32
BF16 = jnp.bfloat16

H = 32
D = 128
SK = 4096
WIN = 1024
M = 640
C = 512
HD = H * D
SCALE = float(D) ** -0.5

KV_GROUPS = 4
HPG = H // KV_GROUPS
CKV_SPLIT = 3072
NSEM = 2 + KV_GROUPS

ZR = 128
ZJ = 8
NZB = (SK - WIN) // ZR
NDB = WIN // ZR
NHG = H // ZJ
S_AWQ = (5, M // 5, HD)
S_WO = (8, HD // 8, M)
S_CKV = (8, SK // 8, C)
S_BWQ = (5, M * H // 5, D)
S_BWU = (8, C * H // 8, D)
AWQ_ROWS, AWQ_COLS = 8, 1024
WO_ROWS = 32
CKV_ROWS = 32
BWQ_ROWS = 64
BWU_ROWS = 64

NT = (((1,), (1,)), ((), ()))


def _dot(a, b):
    return jnp.dot(a, b, preferred_element_type=F32)


def _dot_nt(a, b):
    return lax.dot_general(a, b, NT, preferred_element_type=F32)


def _iota(shape, dim):
    return lax.broadcasted_iota(jnp.int32, shape, dim)


def _colrep(row):
    eye = _iota((128, 128), 0) == _iota((128, 128), 1)
    lhs = jnp.where(eye, jnp.broadcast_to(row, (128, 128)), 0.0).astype(BF16)
    return _dot(lhs, jnp.ones((128, 128), BF16))


def _hi_lo(x):
    hi = x.astype(BF16)
    return jnp.concatenate([hi, (x - hi.astype(F32)).astype(BF16)], axis=0)


def _kernel(
    ax_h, ak_h, av_h, awq_h, awo_h, bx_h, ckv_h, bwq_h, bwuk_h, bwuv_h, bwo_h, g_h,
    out_h, gax_h, gak_h, gav_h, gawq_h, gawo_h, gbx_h, gckv_h, gbwq_h, gbwuk_h, gbwuv_h, gbwo_h,
    ax_v, bx_v, g_v, k_v, v_v, awq_v, awo_v, ckv_v, bwq_v, bwuk_v, bwuv_v, bwo_v,
    out_s, gax_s, gbx_s, z_s, gk_s, gv_s, gawq_s, gawo_s, gckv_s, gbwq_s, gbwuk_s, gbwuv_s, gbwo_s,
    qa_s, doa_s, oa_s, dqa_s, qb_s, dctx_s, ctx_s, dqb_s, row_s, xrep_s, t_s, qd_s, ps_s, latt_s,
    sems,
):
    def rd(src, dst, k):
        return pltpu.make_async_copy(src, dst, sems.at[k])

    rd_first = [rd(awq_h, awq_v, 0), rd(ax_h, ax_v, 0), rd(bx_h, bx_v, 0), rd(g_h, g_v, 0)]
    rd_awo = rd(awo_h, awo_v, 1)
    rd_kv = []
    for gi in range(KV_GROUPS):
        hs = pl.ds(gi * HPG, HPG)
        rd_kv.append([rd(ak_h.at[hs, pl.ds(SK - WIN, WIN), :], k_v.at[hs], 2 + gi),
                      rd(av_h.at[hs, pl.ds(SK - WIN, WIN), :], v_v.at[hs], 2 + gi)])
    rd_bwq = rd(bwq_h, bwq_v, 0)
    rd_bwo = rd(bwo_h, bwo_v, 1)
    rd_bwuk = rd(bwuk_h, bwuk_v, 2)
    rd_bwuv = [rd(bwuv_h, bwuv_v, 3),
               rd(ckv_h.at[pl.ds(0, CKV_SPLIT)], ckv_v.at[pl.ds(0, CKV_SPLIT)], 3)]
    rd_ckv1 = rd(ckv_h.at[pl.ds(CKV_SPLIT, SK - CKV_SPLIT)],
                 ckv_v.at[pl.ds(CKV_SPLIT, SK - CKV_SPLIT)], 4)

    wsem = sems.at[0]

    def zero_copy(dst_h, i):
        h0 = (i // NZB) * ZJ
        r0 = pl.multiple_of((i % NZB) * ZR, ZR)
        return pltpu.make_async_copy(z_s, dst_h.at[pl.ds(h0, ZJ), pl.ds(r0, ZR), :], wsem)

    def cache_copy(src, dst_h, i):
        h0 = (i // NDB) * ZJ
        r0 = pl.multiple_of((i % NDB) * ZR, ZR)
        return pltpu.make_async_copy(
            src.at[pl.ds(h0, ZJ), pl.ds(r0, ZR), :],
            dst_h.at[pl.ds(h0, ZJ), pl.ds(pl.multiple_of(SK - WIN + r0, ZR), ZR), :], wsem)

    def rows_copy(src, dst_h, rows):
        def mk(i):
            r0 = pl.multiple_of(i * rows, rows)
            return pltpu.make_async_copy(src.at[:, pl.ds(r0, rows), :], dst_h.at[:, pl.ds(r0, rows), :], wsem)
        return mk, src.shape[1] // rows

    awq_nc = HD // AWQ_COLS

    def awq_copy(i):
        r0 = pl.multiple_of((i // awq_nc) * AWQ_ROWS, AWQ_ROWS)
        c0 = pl.multiple_of((i % awq_nc) * AWQ_COLS, AWQ_COLS)
        return pltpu.make_async_copy(gawq_s.at[:, pl.ds(r0, AWQ_ROWS), pl.ds(c0, AWQ_COLS)],
                                     gawq_h.at[:, pl.ds(r0, AWQ_ROWS), pl.ds(c0, AWQ_COLS)], wsem)

    writes = {
        "zk": (lambda i: zero_copy(gak_h, i), NHG * NZB),
        "zv": (lambda i: zero_copy(gav_h, i), NHG * NZB),
        "gk": (lambda i: cache_copy(gk_s, gak_h, i), NHG * NDB),
        "gv": (lambda i: cache_copy(gv_s, gav_h, i), NHG * NDB),
        "gckv": rows_copy(gckv_s, gckv_h, CKV_ROWS),
        "gbwuk": rows_copy(gbwuk_s, gbwuk_h, BWU_ROWS),
        "gbwuv": rows_copy(gbwuv_s, gbwuv_h, BWU_ROWS),
        "gbwo": rows_copy(gbwo_s, gbwo_h, WO_ROWS),
        "gbwq": rows_copy(gbwq_s, gbwq_h, BWQ_ROWS),
        "gawo": rows_copy(gawo_s, gawo_h, WO_ROWS),
        "gawq": (awq_copy, (S_AWQ[1] // AWQ_ROWS) * awq_nc),
    }
    small_writes = [
        pltpu.make_async_copy(out_s, out_h, wsem),
        pltpu.make_async_copy(gax_s, gax_h, wsem),
        pltpu.make_async_copy(gbx_s, gbx_h, wsem),
    ]
    issued = {name: 0 for name in writes}

    def issue(name, count=None):
        mk, n = writes[name]
        lo = issued[name]
        hi = n if count is None else lo + count
        assert lo < hi <= n
        issued[name] = hi

        def body(i, carry):
            mk(i).start()
            return carry
        lax.fori_loop(lo, hi, body, 0)

    early = ("zk", "zv", "gk", "gv")

    def top_up(count):
        for name in early:
            k = min(count, writes[name][1] - issued[name])
            if k > 0:
                issue(name, k)
                count -= k

    def wait_writes(name):
        mk, n = writes[name]
        assert issued[name] == n

        def body(i, carry):
            mk(i).wait()
            return carry
        lax.fori_loop(0, n, body, 0)

    def xa():
        return ax_v[0].astype(F32)

    def xb():
        return bx_v[0].astype(F32)

    def ga():
        return g_v[0][:, :M].astype(F32)

    def gb():
        return g_v[0][:, M:].astype(F32)

    def put_rows(dst, r, n, val, cols=slice(None)):
        rps = dst.shape[1]
        dst[r // rps, pl.ds(pl.multiple_of(r % rps, n), n), cols] = val

    def rows16(row):
        return jnp.broadcast_to(row, (16, row.shape[1])).astype(BF16)

    def row_to_heads(row, dst):
        for h in range(H):
            dst[h:h + 1, :] = row[0:1, h * D:(h + 1) * D]

    def heads_to_row(src):
        for h in range(H):
            row_s[:, h * D:(h + 1) * D] = jnp.broadcast_to(src[h:h + 1, :], (16, D)).astype(BF16)
        return row_s[...]

    def fill_xrep(x):
        for t in range(M // 128):
            xrep_s[t * 128:(t + 1) * 128, :] = _colrep(x[:, t * 128:(t + 1) * 128])

    def outer_wo(src, grow, dst):
        def body(h, carry):
            col = _colrep(src[pl.ds(h, 1), :])
            for t in range(M // 128):
                cols = slice(t * 128, (t + 1) * 128)
                put_rows(dst, h * D, D, (col * grow[:, cols]).astype(BF16), cols)
            return carry
        lax.fori_loop(0, H, body, 0)

    def a_q():
        row_to_heads(_dot(rows16(xa()), awq_v[...]), qa_s)

    def a_do():
        row_to_heads(_dot_nt(rows16(ga()), awo_v[...]), doa_s)

    def a_head(h, carry):
        kk = k_v[h]
        vv = v_v[h]
        q = qa_s[pl.ds(h, 1), :]
        do = doa_s[pl.ds(h, 1), :]
        s = _dot_nt(kk, jnp.broadcast_to(q, (D, D)).astype(BF16)) * SCALE
        dp = _dot_nt(vv, jnp.broadcast_to(do, (D, D)).astype(BF16))
        e = jnp.exp(s - jnp.max(s, axis=0, keepdims=True))
        inv = 1.0 / jnp.sum(e, axis=0, keepdims=True)
        u = e * (dp - jnp.sum(e * dp, axis=0, keepdims=True) * inv)
        f = inv * SCALE
        gk_s[h] = (u * (q * f)).astype(BF16)
        gv_s[h] = (e * (do * inv)).astype(BF16)
        oa_s[pl.ds(h, 1), :] = jnp.sum(e * vv.astype(F32), axis=0, keepdims=True) * inv
        dqa_s[pl.ds(h, 1), :] = jnp.sum(u * kk.astype(F32), axis=0, keepdims=True) * f
        return carry

    def a_out():
        out_s[0, :, 0:M] = _dot(heads_to_row(oa_s), awo_v[...])[0:1].astype(BF16)

    def a_dwo():
        outer_wo(oa_s, ga(), gawo_s)

    def a_dx():
        gax_s[0] = _dot_nt(heads_to_row(dqa_s), awq_v[...])[0:1].astype(BF16)

    def a_dwq():
        fill_xrep(xa())
        for h in range(H):
            blk = (xrep_s[...] * dqa_s[h:h + 1, :]).astype(BF16)
            gawq_s[:, :, h * D:(h + 1) * D] = blk.reshape(S_AWQ[0], S_AWQ[1], D)

    def b_q():
        fill_xrep(xb())

        def body(i, acc):
            for j in range(8):
                m = i * 8 + j
                w = bwq_v[pl.ds(pl.multiple_of(m * H, H), H), :].astype(F32)
                acc = acc + w * xrep_s[pl.ds(m, 1), :]
            return acc
        qb_s[...] = lax.fori_loop(0, M // 8, body, jnp.zeros((H, D), F32))

    def b_dctx():
        row_to_heads(_dot_nt(rows16(gb()), bwo_v[...]), dctx_s)

    def b_absorb(w_v, vec_s, first):
        cb = 16
        diag = (_iota((cb * H, D), 0) % H) == (_iota((cb * H, D), 1) % H)
        zpad = jnp.zeros((H, D), F32)
        parts = [vec_s[...], zpad, zpad, zpad] if first else [zpad, vec_s[...], zpad, zpad]
        rhs = jnp.concatenate(parts, axis=0).astype(BF16)

        def body(i, carry):
            r0 = pl.multiple_of(i * cb * H, cb * H)
            r = _dot_nt(w_v[pl.ds(r0, cb * H), :], rhs)
            r = jnp.sum(jnp.where(diag, r, 0.0).reshape(cb, H, D), axis=1)
            t0 = pl.multiple_of(i * cb, cb)
            if first:
                t_s[pl.ds(t0, cb), :] = r
            else:
                t_s[pl.ds(t0, cb), :] = t_s[pl.ds(t0, cb), :] + r
            return carry
        lax.fori_loop(0, C // cb, body, 0)

    def b_qd():
        qd_s[...] = _hi_lo(t_s[0:C, :].T[0:2 * H])

    def b_attn():
        sd = _dot_nt(qd_s[...], ckv_v[...])
        sd = sd[0:2 * H] + sd[2 * H:4 * H]
        s = sd[0:H] * SCALE
        dp = sd[H:2 * H]
        e = jnp.exp(s - jnp.max(s, axis=1, keepdims=True))
        p = e * (1.0 / jnp.sum(e, axis=1, keepdims=True))
        ds = p * (dp - jnp.sum(p * dp, axis=1, keepdims=True)) * SCALE
        ps_s[0:H, :] = ds
        ps_s[H:2 * H, :] = p
        ps_s[2 * H:4 * H, :] = jnp.zeros((2 * H, SK), F32)
        lat = _dot(ps_s[0:2 * H, :].astype(BF16), ckv_v[...])
        latt_s[...] = _hi_lo(lat).astype(F32).T

    def b_dckv():
        def body(j, carry):
            k0 = pl.multiple_of(j * 512, 512)
            pst = ps_s[:, pl.ds(k0, 512)].T.astype(BF16)
            put_rows(gckv_s, j * 512, 512, _dot(pst, qd_s[...]).astype(BF16))
            return carry
        lax.fori_loop(0, SK // 512, body, 0)

    def b_lat():
        cc = 8
        sel = (_iota((cc * H, D), 0) % H) == (_iota((cc * H, D), 1) % H)
        jj = _iota((D, 2 * D), 0)
        nn = _iota((D, 2 * D), 1)
        expand = jnp.where((jj % (2 * H) < H) == (nn < D), 1.0, 0.0).astype(BF16)
        qb_t = jnp.concatenate([qb_s[...]] * cc, axis=0)
        dctx_t = jnp.concatenate([dctx_s[...]] * cc, axis=0)

        def body(i, carry):
            dq_acc, ctx_acc = carry
            c0 = i * cc
            lhs = jnp.concatenate(
                [jnp.broadcast_to(latt_s[pl.ds(c0 + j, 1), :], (H, D)) for j in range(cc)], axis=0)
            rep = _dot(jnp.where(sel, lhs, 0.0).astype(BF16), expand)
            rep_ds = rep[:, 0:D]
            rep_p = rep[:, D:2 * D]
            put_rows(gbwuk_s, c0 * H, cc * H, (rep_ds * qb_t).astype(BF16))
            put_rows(gbwuv_s, c0 * H, cc * H, (rep_p * dctx_t).astype(BF16))
            r0 = pl.multiple_of(c0 * H, cc * H)
            wk = bwuk_v[pl.ds(r0, cc * H), :].astype(F32)
            wv = bwuv_v[pl.ds(r0, cc * H), :].astype(F32)
            dq_acc = dq_acc + jnp.sum((rep_ds * wk).reshape(cc, H, D), axis=0)
            ctx_acc = ctx_acc + jnp.sum((rep_p * wv).reshape(cc, H, D), axis=0)
            return dq_acc, ctx_acc

        dqb, ctx = lax.fori_loop(0, C // cc, body, (jnp.zeros((H, D), F32), jnp.zeros((H, D), F32)))
        ctx_s[...] = ctx
        dqb_s[...] = dqb

    def b_out():
        out_s[0, :, M:2 * M] = _dot(heads_to_row(ctx_s), bwo_v[...])[0:1].astype(BF16)

    def b_dwo():
        outer_wo(ctx_s, gb(), gbwo_s)

    def b_dwq():
        def body(i, carry):
            dq = dqb_s[...]
            for j in range(8):
                m = i * 8 + j
                w = bwq_v[pl.ds(pl.multiple_of(m * H, H), H), :].astype(F32) * dq
                t_s[pl.ds(m, 1), :] = jnp.sum(w, axis=0, keepdims=True)
                put_rows(gbwq_s, m * H, H, (xrep_s[pl.ds(m, 1), :] * dq).astype(BF16))
            return carry
        lax.fori_loop(0, M // 8, body, 0)
        gbx_s[0] = jnp.sum(t_s[...].T, axis=0, keepdims=True).astype(BF16)

    for cp in rd_first:
        cp.start()
    rd_awo.start()
    for pair in rd_kv:
        for cp in pair:
            cp.start()
    z_s[...] = jnp.zeros(z_s.shape, BF16)

    for cp in rd_first:
        cp.wait()
    rd_bwq.start()
    a_q()
    rd_awo.wait()
    rd_bwo.start()
    a_do()
    for gi in range(KV_GROUPS):
        for cp in rd_kv[gi]:
            cp.wait()
        if gi == 0:
            rd_bwuk.start()
        elif gi == 1:
            for cp in rd_bwuv:
                cp.start()
        elif gi == 2:
            rd_ckv1.start()
        lax.fori_loop(gi * HPG, (gi + 1) * HPG, a_head, 0)
    rd_bwq.wait()
    rd_bwo.wait()
    rd_bwuk.wait()
    for cp in rd_bwuv:
        cp.wait()

    top_up(72)
    b_q()
    b_dctx()
    top_up(12)
    b_absorb(bwuk_v, qb_s, True)
    top_up(18)
    b_absorb(bwuv_v, dctx_s, False)
    b_qd()
    top_up(19)
    rd_ckv1.wait()
    b_attn()
    top_up(14)
    b_dckv()
    top_up(13)
    b_lat()
    top_up(35)
    b_out()
    b_dwo()
    top_up(18)
    b_dwq()
    top_up(16)
    a_out()
    a_dwo()
    top_up(18)
    a_dx()
    a_dwq()
    top_up(H * SK)
    for cp in small_writes:
        cp.start()
    late = ("gckv", "gbwuk", "gbwuv", "gbwo", "gbwq", "gawo", "gawq")
    for name in late:
        issue(name)

    for name in early:
        wait_writes(name)
    for cp in small_writes:
        cp.wait()
    for name in late:
        wait_writes(name)


@jax.jit
def pallas_concat_heads__sliding_block_cached__compressed_kv_cla__decode_kernel(
    A_x: jax.Array,
    A_k_cache: jax.Array,
    A_v_cache: jax.Array,
    A_wq: jax.Array,
    A_wo: jax.Array,
    B_x: jax.Array,
    B_c_kv: jax.Array,
    B_w_q: jax.Array,
    B_w_uk: jax.Array,
    B_w_uv: jax.Array,
    B_w_o: jax.Array,
    grad_out: jax.Array,
):
    sds = jax.ShapeDtypeStruct
    out_shape = (
        sds((1, 1, 2 * M), BF16),
        sds((1, 1, M), BF16),
        sds((H, SK, D), BF16),
        sds((H, SK, D), BF16),
        sds(S_AWQ, BF16),
        sds(S_WO, BF16),
        sds((1, 1, M), BF16),
        sds(S_CKV, BF16),
        sds(S_BWQ, BF16),
        sds(S_BWU, BF16),
        sds(S_BWU, BF16),
        sds(S_WO, BF16),
    )
    vm = pltpu.VMEM
    scratch = [
        vm((1, 1, M), BF16), vm((1, 1, M), BF16), vm((1, 1, 2 * M), BF16),
        vm((H, WIN, D), BF16), vm((H, WIN, D), BF16),
        vm((M, HD), BF16), vm((HD, M), BF16),
        vm((SK, C), BF16),
        vm((M * H, D), BF16), vm((C * H, D), BF16), vm((C * H, D), BF16), vm((HD, M), BF16),
        vm((1, 1, 2 * M), BF16), vm((1, 1, M), BF16), vm((1, 1, M), BF16),
        vm((ZJ, ZR, D), BF16),
        vm((H, WIN, D), BF16), vm((H, WIN, D), BF16),
        vm(S_AWQ, BF16), vm(S_WO, BF16), vm(S_CKV, BF16),
        vm(S_BWQ, BF16), vm(S_BWU, BF16), vm(S_BWU, BF16), vm(S_WO, BF16),
        vm((H, D), F32), vm((H, D), F32), vm((H, D), F32), vm((H, D), F32),
        vm((H, D), F32), vm((H, D), F32), vm((H, D), F32), vm((H, D), F32),
        vm((16, HD), BF16), vm((M, D), F32),
        vm((M, D), F32), vm((D, C), BF16), vm((D, SK), F32), vm((C, D), F32),
        pltpu.SemaphoreType.DMA((NSEM,)),
    ]
    any_spec = pl.BlockSpec(memory_space=pl.ANY)
    outs = pl.pallas_call(
        _kernel,
        out_shape=out_shape,
        in_specs=[any_spec] * 12,
        out_specs=(any_spec,) * 12,
        scratch_shapes=scratch,
        compiler_params=pltpu.CompilerParams(vmem_limit_bytes=120 * 1024 * 1024),
        name="fused_decode_fwd_bwd",
    )(
        A_x,
        A_k_cache.reshape(H, SK, D),
        A_v_cache.reshape(H, SK, D),
        A_wq,
        A_wo,
        B_x,
        B_c_kv.reshape(SK, C),
        B_w_q.reshape(M * H, D),
        B_w_uk.reshape(C * H, D),
        B_w_uv.reshape(C * H, D),
        B_w_o.reshape(HD, M),
        grad_out,
    )
    (out, gax, gak, gav, gawq, gawo, gbx, gckv, gbwq, gbwuk, gbwuv, gbwo) = outs
    return (
        out,
        gax,
        gak.reshape(1, H, SK, D),
        gav.reshape(1, H, SK, D),
        gawq.reshape(M, HD),
        gawo.reshape(HD, M),
        gbx,
        gckv.reshape(1, SK, C),
        gbwq.reshape(M, H, D),
        gbwuk.reshape(C, H, D),
        gbwuv.reshape(C, H, D),
        gbwo.reshape(H, D, M),
    )
```
